```python
import os as _os
_os.environ.setdefault('JAX_PLATFORMS', 'cpu')
import jax
import jax.numpy as jnp

def _softmax(x, axis=-1):
    return jax.nn.softmax(x, axis=axis)

def _gelu(x):
    return jax.nn.gelu(x, approximate=True)

def _silu(x):
    return jax.nn.silu(x)

def _sigmoid(x):
    return jax.nn.sigmoid(x)

def _layernorm(x, axis=-1, eps=1e-05):
    m = jnp.mean(x, axis=axis, keepdims=True)
    v = jnp.var(x, axis=axis, keepdims=True)
    return (x - m) / jnp.sqrt(v + eps)

def _scatter_add(tgt, idx, src, axis=0):
    return tgt.at[idx].add(src)

def _segment_sum(src, seg, n):
    return jax.ops.segment_sum(src, seg, n)

class _Rng:

    def __init__(self, key):
        self._k = key

    def _next(self):
        self._k, sub = jax.random.split(self._k)
        return sub

    def normal(self, shape):
        return jax.random.normal(self._next(), shape, dtype=jnp.bfloat16)

    def randint(self, lo, hi, shape):
        return jax.random.randint(self._next(), shape, lo, hi, dtype=jnp.int32)

    def uniform(self, shape, lo=0.0, hi=1.0):
        return jax.random.uniform(self._next(), shape, jnp.bfloat16, lo, hi)

    def permutation(self, n):
        return jax.random.permutation(self._next(), n)
kernel_name = 'parallel_sum__memory_aug_recurrent_mem_tr__dense_activation_silu__prompt'

def setup_inputs():
    _rng = _Rng(jax.random.key(int.from_bytes(__import__("os").urandom(4), "little")))
    _w = lambda a: (lambda t: t.astype(jnp.bfloat16) if jnp.issubdtype(t.dtype, jnp.floating) else t)(jnp.asarray(a))

    def _A_setup():
        B, S, Dm = (1, 2048, 448)
        H, Dh = (16, 256)
        M, seg = (8, 32)
        seg = min(seg, S)
        S = S // seg * seg
        return {'x': _w((lambda *s: _rng.normal(s) * 0.05)(B, S, Dm)), 'mem0': _w((lambda *s: _rng.normal(s) * 0.2)(B, M, Dm)), 'Wq': _w((lambda *s: _rng.normal(s) * 0.8)(Dm, H, Dh) * Dm ** (-0.5)), 'Wk': _w((lambda *s: _rng.normal(s) * 0.8)(Dm, H, Dh) * Dm ** (-0.5)), 'Wv': _w((lambda *s: _rng.normal(s) * 0.2)(Dm, H, Dh) * Dm ** (-0.5)), 'Wo': _w((lambda *s: _rng.normal(s) * 0.2)(H, Dh, Dm) * (H * Dh) ** (-0.5)), 'seg_len': seg}
    _A_in = _A_setup()

    def _B_setup():
        B, S, D, F = (1, 2048, 448, 1792)
        return {'x': _w((lambda *s: _rng.normal(s) * 0.05)(B, S, D)), 'w1': _w((lambda *s: _rng.normal(s) * 0.05)(D, F) * D ** (-0.5)), 'w2': _w((lambda *s: _rng.normal(s) * 0.05)(F, D) * F ** (-0.5))}
    _B_in = _B_setup()
    return {'A_x': _A_in['x'], 'A_mem0': _A_in['mem0'], 'A_Wq': _A_in['Wq'], 'A_Wk': _A_in['Wk'], 'A_Wv': _A_in['Wv'], 'A_Wo': _A_in['Wo'], 'A_seg_len': _A_in['seg_len'], 'B_x': _B_in['x'], 'B_w1': _B_in['w1'], 'B_w2': _B_in['w2']}

def reference(A_x, A_mem0, A_Wq, A_Wk, A_Wv, A_Wo, A_seg_len, B_x, B_w1, B_w2):

    def _A_ref(x, mem0, Wq, Wk, Wv, Wo, seg_len):
        B, S, Dm = x.shape
        H, Dh = (Wq.shape[1], Wq.shape[2])
        M = mem0.shape[1]
        scale = Dh ** (-0.5)
        n_seg = S // seg_len
        L = M + seg_len
        idx = jnp.arange(L)
        mask = (idx[:, None] < M) | (idx[:, None] >= idx[None, :])
        mem = mem0
        outs = []
        for s in range(n_seg):
            xs = x[:, s * seg_len:(s + 1) * seg_len, :].copy()
            h = jnp.concatenate([mem, xs], axis=1)
            q = jnp.einsum('btd,dhe->bhte', h, Wq)
            k = jnp.einsum('btd,dhe->bhte', h, Wk)
            v = jnp.einsum('btd,dhe->bhte', h, Wv)
            scores = jnp.einsum('bhqe,bhke->bhqk', q, k) * scale
            scores = jnp.where(mask[None, None], scores, -1000000000.0)
            p = _softmax(scores, axis=-1)
            o = jnp.einsum('bhqk,bhke->bhqe', p, v)
            o = jnp.einsum('bhte,hed->btd', o, Wo)
            mem = o[:, :M, :].copy()
            outs.append(o[:, M:, :])
        return jnp.concatenate(outs, axis=1)

    def _B_ref(x, w1, w2):
        h = jnp.einsum('bsd,df->bsf', x, w1)
        h = _silu(h)
        out = jnp.einsum('bsf,fd->bsd', h, w2)
        return out
    x = A_x
    xn = _layernorm(x, axis=-1)
    return x + _A_ref(xn, A_mem0, A_Wq, A_Wk, A_Wv, A_Wo, A_seg_len) + _B_ref(xn, B_w1, B_w2)
```

```python
import functools
import jax, jax.numpy as jnp, numpy as np
from jax.experimental import pallas as pl
from jax.experimental.pallas import tpu as pltpu

D = 448; DP = 512; H = 16; DH = 256; F = 1792; SEG = 32; MEM = 8; S = 2048
f32 = jnp.float32; bf16 = jnp.bfloat16; u32 = jnp.uint32
NEG = -1e9
NT = (((1,), (1,)), ((), ()))

def _stack(Y, groups):
    outs = []
    for g in groups:
        rows = Y[8*g:8*g+8, :]
        tiles = []
        for m in range(8):
            R = rows[:, 6144 + 128*m: 6144 + 128*(m+1)]
            Ro = pltpu.roll(R, 64, 1)
            for h, rr in ((2*m, R), (2*m+1, Ro)):
                tiles.append(jnp.concatenate([rows[:, 384*h:384*(h+1)], rr], axis=1))
        outs.append(jnp.concatenate(tiles, axis=0))
    return outs

def _group_allreduce(x, op):
    lane = jax.lax.broadcasted_iota(jnp.int32, x.shape, 1)
    for r in (4, 2, 1):
        a = pltpu.roll(x, r, 1)
        b = pltpu.roll(x, 128 - r, 1)
        x = op(x, jnp.where((lane & r) != 0, a, b))
    return x

def _softmax_tiles(Sc):
    sub = jax.lax.broadcasted_iota(jnp.int32, (8, 128), 0)
    lane = jax.lax.broadcasted_iota(jnp.int32, (8, 128), 1)
    tri = (lane & 7) <= sub
    def vis(q, t):
        if q == 0 or t == 0 or t < q: return 1
        if t == q: return 2
        return 0
    T = {}; ms = []
    for q in range(5):
        m = None
        for t in range(5):
            v = vis(q, t)
            if v == 0: continue
            s = Sc[8*q:8*q+8, 128*t:128*(t+1)]
            if v == 2:
                s = jnp.where(tri, s, NEG)
            T[q, t] = s
            m = s if m is None else jnp.maximum(m, s)
        ms.append(m)
    Mx = _group_allreduce(jnp.concatenate(ms, axis=0), jnp.maximum)
    E = {}; sums = []
    for q in range(5):
        mq = Mx[8*q:8*q+8]
        sm = None
        for t in range(5):
            if (q, t) in T:
                e = jnp.exp(T[q, t] - mq)
                E[q, t] = e
                sm = e if sm is None else sm + e
        sums.append(sm)
    inv = 1.0 / _group_allreduce(jnp.concatenate(sums, axis=0), jnp.add)
    rows = []
    z = jnp.zeros((8, 128), f32)
    for q in range(5):
        iq = inv[8*q:8*q+8]
        rows.append(jnp.concatenate([E[q, t] * iq if (q, t) in E else z for t in range(5)], axis=1))
    rows.append(jnp.zeros((8, 640), f32))
    return jnp.concatenate(rows, axis=0).astype(bf16)

def _w(ref):
    return pltpu.bitcast(ref[...], bf16)

def _deinterleave(buf, m):
    w32 = buf.bitcast(u32)
    los, his = [], []
    for eh in range(2):
        a = w32[eh, pl.ds(m, D // 2, stride=16), :]
        b = w32[eh, pl.ds(m + 8, D // 2, stride=16), :]
        los.append((a & jnp.uint32(0xFFFF)) | (b << 16))
        his.append((a >> 16) | (b & jnp.uint32(0xFFFF0000)))
    return (pltpu.bitcast(jnp.concatenate(los, axis=1), bf16), pltpu.bitcast(jnp.concatenate(his, axis=1), bf16))

def _store_pair(dst, m, A0, A1):
    b0 = A0.astype(bf16); b1 = A1.astype(bf16)
    dst[:, 384*(2*m):384*(2*m+1)] = pltpu.bitcast(b0[:, 0:384], u32)
    dst[:, 384*(2*m+1):384*(2*m+2)] = pltpu.bitcast(b1[:, 0:384], u32)
    rem = jnp.concatenate([A0[:, 384:448], A1[:, 384:448]], axis=1).astype(bf16)
    dst[:, 6144 + 128*m: 6144 + 128*(m+1)] = pltpu.bitcast(rem, u32)

def kernel(xT_hbm, mem_ref, wq_hbm, wk_hbm, wv_hbm, woT_hbm, w1_hbm, w2T_hbm, outT_hbm,
           xT_s, xn_s, wq_s, wk_s, wv_s, woT_s, w1_s, w2T_s, WK, WV, W1, W2, R_s, outT_s, sem, *, order):
    def cp(src, dst, k):
        return pltpu.make_async_copy(src, dst, sem.at[k])
    copies = {
        'q0': cp(wq_hbm.at[:, 0:128], wq_s.at[0], 0), 'q1': cp(wq_hbm.at[:, 128:256], wq_s.at[1], 1),
        'k0': cp(wk_hbm.at[:, 0:128], wk_s.at[0], 2), 'k1': cp(wk_hbm.at[:, 128:256], wk_s.at[1], 3),
        'v0': cp(wv_hbm.at[:, 0:128], wv_s.at[0], 4), 'v1': cp(wv_hbm.at[:, 128:256], wv_s.at[1], 5),
        'o': cp(woT_hbm, woT_s, 6), 'x': cp(xT_hbm, xT_s, 7), 'w1': cp(w1_hbm, w1_s, 8), 'w2': cp(w2T_hbm, w2T_s, 9),
    }
    for k in ('q0', 'q1', 'k0', 'k1', 'x', 'v0', 'v1', 'o', 'w1', 'w2'):
        copies[k].start()
    for k in ('q0', 'q1', 'k0', 'k1'):
        copies[k].wait()
    for m in range(8):
        q0, q1 = _deinterleave(wq_s, m)
        k0, k1 = _deinterleave(wk_s, m)
        A0 = jax.lax.dot_general(k0, q0, NT, preferred_element_type=f32) * (DH ** -0.5)
        A1 = jax.lax.dot_general(k1, q1, NT, preferred_element_type=f32) * (DH ** -0.5)
        _store_pair(WK, m, A0, A1)
    copies['x'].wait()
    for c in range(S // 128):
        xb = xT_s[:, 128*c:128*(c+1)].astype(f32)
        mu = jnp.mean(xb, axis=0, keepdims=True)
        xc = xb - mu
        var = jnp.mean(xc * xc, axis=0, keepdims=True)
        xnT = xc * jax.lax.rsqrt(var + 1e-5)
        xn_s[128*c:128*(c+1), :] = jnp.concatenate([xnT, jnp.zeros((DP - D, 128), f32)], axis=0).T
    for k in ('v0', 'v1', 'o'):
        copies[k].wait()
    for m in range(8):
        v0, v1 = _deinterleave(wv_s, m)
        U0 = jax.lax.dot_general(v0, woT_s[2*m], NT, preferred_element_type=f32)
        U1 = jax.lax.dot_general(v1, woT_s[2*m+1], NT, preferred_element_type=f32)
        _store_pair(WV, m, U0, U1)
    copies['w1'].wait()
    W1[...] = pltpu.bitcast(w1_s[...], u32)
    copies['w2'].wait()
    W2[...] = pltpu.bitcast(w2T_s[...].T, u32)

    def mlp_up(xb):
        h = jnp.dot(xb, _w(W1), preferred_element_type=f32)
        return (h * jax.nn.sigmoid(h)).astype(bf16)
    def mlp_down(hb):
        return jnp.dot(hb, _w(W2), preferred_element_type=f32)

    def body(p, mem):
        r0 = pl.multiple_of(p * 64, 64)
        xn = xn_s[pl.ds(r0, 64), :]
        hB = jnp.concatenate([mem, xn[0:40]], axis=0).astype(bf16)
        lhsB = hB[:, 0:D]
        YK = jnp.dot(lhsB, _w(WK), preferred_element_type=f32)
        if order == 1: hidB = mlp_up(xn[0:32, 0:D].astype(bf16))
        sk = _stack(YK, range(6))
        kkB = jnp.concatenate(sk[0:5], axis=0).astype(bf16)
        Sc = jax.lax.dot_general(hB, kkB, NT, preferred_element_type=f32)
        YV = jnp.dot(lhsB, _w(WV), preferred_element_type=f32)
        P = _softmax_tiles(Sc)
        sv = _stack(YV, range(6))
        voB = jnp.concatenate(sv[0:5], axis=0).astype(bf16)
        oB = jnp.dot(P, voB, preferred_element_type=f32)
        if order == 0: hidB = mlp_up(xn[0:32, 0:D].astype(bf16))
        mlpB = mlp_down(hidB)
        R_s[pl.ds(r0, 32), :] = oB[8:40, 0:D] + mlpB
        lane = jax.lax.broadcasted_iota(jnp.int32, (8, DP), 1)
        mem1 = jnp.where(lane < D, oB[0:8], 0.0)
        hA = jnp.concatenate([mem1, xn[40:64]], axis=0).astype(bf16)
        lhsA = hA[:, 0:D]
        hqA = jnp.concatenate([mem1, xn[32:64], jnp.zeros((8, DP), f32)], axis=0).astype(bf16)
        YK2 = jnp.dot(lhsA, _w(WK), preferred_element_type=f32)
        if order == 1: hidA = mlp_up(xn[32:64, 0:D].astype(bf16))
        sk2 = _stack(YK2, range(4))
        kkA = jnp.concatenate([sk2[0], sk[5], sk2[1], sk2[2], sk2[3]], axis=0).astype(bf16)
        Sc2 = jax.lax.dot_general(hqA, kkA, NT, preferred_element_type=f32)
        YV2 = jnp.dot(lhsA, _w(WV), preferred_element_type=f32)
        P2 = _softmax_tiles(Sc2)
        sv2 = _stack(YV2, range(4))
        voA = jnp.concatenate([sv2[0], sv[5], sv2[1], sv2[2], sv2[3]], axis=0).astype(bf16)
        oA = jnp.dot(P2, voA, preferred_element_type=f32)
        if order == 0: hidA = mlp_up(xn[32:64, 0:D].astype(bf16))
        mlpA = mlp_down(hidA)
        R_s[pl.ds(r0 + 32, 32), :] = oA[8:40, 0:D] + mlpA
        return jnp.where(lane < D, oA[0:8], 0.0)
    mem0 = jnp.concatenate([mem_ref[...].astype(f32), jnp.zeros((MEM, DP - D), f32)], axis=1)
    jax.lax.fori_loop(0, S // 64, body, mem0)
    outs = []
    for c in range(S // 128):
        rb = R_s[128*c:128*(c+1), :]
        rT = jnp.concatenate([rb, jnp.zeros((128, DP - D), f32)], axis=1).T[0:D]
        outT_s[:, 128*c:128*(c+1)] = (xT_s[:, 128*c:128*(c+1)].astype(f32) + rT).astype(bf16)
        co = cp(outT_s.at[:, 128*c:128*(c+1)], outT_hbm.at[:, 128*c:128*(c+1)], 10 + c)
        co.start(); outs.append(co)
    for co in outs:
        co.wait()

def make(order=0):
    def run(A_x, A_mem0, A_Wq, A_Wk, A_Wv, A_Wo, B_w1, B_w2):
        xT = jnp.swapaxes(A_x[0], 0, 1)
        any_spec = pl.BlockSpec(memory_space=pl.ANY)
        outT = pl.pallas_call(functools.partial(kernel, order=order),
            out_shape=jax.ShapeDtypeStruct((D, S), bf16),
            in_specs=[any_spec, pl.BlockSpec(memory_space=pltpu.VMEM)] + [any_spec]*6,
            out_specs=any_spec,
            scratch_shapes=[
                pltpu.VMEM((D, S), bf16), pltpu.VMEM((S, DP), f32),
                pltpu.VMEM((2, D*H, 128), bf16), pltpu.VMEM((2, D*H, 128), bf16), pltpu.VMEM((2, D*H, 128), bf16),
                pltpu.VMEM((H, D, DH), bf16), pltpu.VMEM((D, F), bf16), pltpu.VMEM((D, F), bf16),
                pltpu.VMEM((D//2, 7168), u32), pltpu.VMEM((D//2, 7168), u32), pltpu.VMEM((D//2, F), u32), pltpu.VMEM((F//2, D), u32),
                pltpu.VMEM((S, D), f32), pltpu.VMEM((D, S), bf16),
                pltpu.SemaphoreType.DMA((10 + S//128,)),
            ],
            compiler_params=pltpu.CompilerParams(vmem_limit_bytes=100*1024*1024),
        )(xT, A_mem0[0], A_Wq.reshape(D*H, DH), A_Wk.reshape(D*H, DH), A_Wv.reshape(D*H, DH),
          jnp.swapaxes(A_Wo, 1, 2), B_w1, jnp.swapaxes(B_w2, 0, 1))
        return jnp.swapaxes(outT, 0, 1)[None]
    return run


@jax.jit
def pallas_parallel_sum__memory_aug_recurrent_mem_tr__dense_activation_silu__prompt_kernel(
    A_x, A_mem0, A_Wq, A_Wk, A_Wv, A_Wo, A_seg_len, B_x, B_w1, B_w2,
):
    del A_seg_len, B_x
    return make(order=0)(A_x, A_mem0, A_Wq, A_Wk, A_Wv, A_Wo, B_w1, B_w2)
```

```python
import jax
import jax.numpy as jnp
from jax.experimental import pallas as pl
from jax.experimental.pallas import tpu as pltpu

D = 448; DP = 512; DU = 384; H = 16; DH = 256; F = 1792; MEM = 8; S = 2048
BLK = 128; NB = S // BLK
f32 = jnp.float32; bf16 = jnp.bfloat16; u32 = jnp.uint32
SCALE = DH ** -0.5
NEG = -1e9 / SCALE
NT = (((1,), (1,)), ((), ()))
REM = 1024
W1_SPLIT = (0, 384, 1024, F)
FS = 768
V1 = {'A': 2048, 'B': 1536}
V2 = {'A': 5632, 'B': 6144}


def _bf(x):
    return pltpu.bitcast(x, bf16)


def _stack(Y, ngroups):
    outs = []
    for g in range(ngroups):
        rows = Y[8*g:8*g+8, :]
        tiles = []
        for m in range(8):
            R = rows[:, 128*m:128*(m+1)]
            for h, rr in ((2*m, R), (2*m+1, pltpu.roll(R, 64, 1))):
                tiles.append(jnp.concatenate([rows[:, REM + DU*h:REM + DU*(h+1)], rr], axis=1))
        outs.append(jnp.concatenate(tiles, axis=0))
    return outs


def _group_allreduce(x, op):
    lane = jax.lax.broadcasted_iota(jnp.int32, x.shape, 1)
    parts = [x] + [jnp.where((lane & 7) >= r, pltpu.roll(x, r, 1), pltpu.roll(x, 128 - (8 - r), 1)) for r in range(1, 8)]
    while len(parts) > 1:
        parts = [op(parts[i], parts[i + 1]) for i in range(0, len(parts), 2)]
    return parts[0]


def _softmax_pieces(Sa, Sb, Sc, S2):
    sub = jax.lax.broadcasted_iota(jnp.int32, (8, 128), 0)
    lane = jax.lax.broadcasted_iota(jnp.int32, (8, 128), 1)
    tri = (lane & 7) <= sub
    row_a = {0: 0, 1: 16, 2: 24, 3: 32, 4: 40}

    def piece(u, t):
        if t < 2:
            return Sa[row_a[u]:row_a[u]+8, 128*t:128*(t+1)]
        if t < 4:
            return Sb[8*(u-1):8*u, 128*(t-2):128*(t-1)]
        return Sc[8*(u-3):8*(u-2), :]

    T = {}; ms = []
    for u in range(5):
        m = None
        for t in range(5):
            if not (u == 4 or t == 0 or t - 1 <= u):
                continue
            s = piece(u, t) + S2[t][8*u:8*u+8]
            if u < 4 and t - 1 == u:
                s = jnp.where(tri, s, NEG)
            T[u, t] = s
            m = s if m is None else jnp.maximum(m, s)
        ms.append(m)
    Mx = _group_allreduce(jnp.concatenate(ms, axis=0), jnp.maximum)
    E = {}; sums = []
    for u in range(5):
        sm = None
        for t in range(5):
            if (u, t) in T:
                e = jnp.exp((T[u, t] - Mx[8*u:8*u+8]) * SCALE)
                E[u, t] = e
                sm = e if sm is None else sm + e
        sums.append(sm)
    inv = 1.0 / _group_allreduce(jnp.concatenate(sums, axis=0), jnp.add)
    z = jnp.zeros((8, 128), f32)

    def p(u, t):
        return E[u, t] * inv[8*u:8*u+8] if (u, t) in E else z

    Pa = jnp.concatenate([jnp.concatenate([p(0, 0), p(0, 1)], axis=1), jnp.zeros((8, 256), f32)] +
                         [jnp.concatenate([p(u, 0), p(u, 1)], axis=1) for u in (1, 2, 3, 4)], axis=0)
    Pb = jnp.concatenate([jnp.concatenate([p(u, 2), p(u, 3)], axis=1) for u in (1, 2, 3, 4)], axis=0)
    Pc = jnp.concatenate([p(u, 4) for u in (3, 4)], axis=0)
    Pt = [jnp.concatenate([p(u, t) for u in range(5)], axis=0) for t in range(5)]
    return Pa.astype(bf16), Pb.astype(bf16), Pc.astype(bf16), Pt


def _block_transpose(blocks, nout):
    shape = next(x for x in blocks if x is not None).shape
    lane = jax.lax.broadcasted_iota(jnp.int32, shape, 1)
    zero = jnp.zeros(shape, f32)
    cur = list(blocks)
    for s in (1, 2, 4):
        hi = ((lane >> 4) & s) != 0
        nxt = []
        for k in range(8):
            if s == 4 and k >= nout:
                nxt.append(None)
                continue
            a_, b_ = (cur[k], cur[k + s]) if k & s == 0 else (cur[k - s], cur[k])
            if a_ is None and b_ is None:
                nxt.append(None)
            elif k & s == 0:
                nxt.append(jnp.where(hi, zero if b_ is None else pltpu.roll(b_, 16 * s, 1), zero if a_ is None else a_))
            else:
                nxt.append(jnp.where(hi, zero if b_ is None else b_, zero if a_ is None else pltpu.roll(a_, 128 - 16 * s, 1)))
        cur = nxt
    return [zero if x is None else x for x in cur[0:nout]]


def _silu(h):
    return h * pl.reciprocal(1.0 + jnp.exp(-h), approx=True)


def _kernel(xT_hbm, mem_ref, wq_hbm, wk_hbm, wv_hbm, woT_hbm, w1_hbm, w2T_hbm, outT_hbm,
            xT_s, xn_s, raw_s, QD, KD, VD, woT_s, w1_s, w2T_s, WK, WV, W1, W2, R_s, outT_s, HID, KT, WQ, WU,
            sem):
    whbm = (wq_hbm, wk_hbm, wv_hbm)

    def wcopy(i, eh):
        return pltpu.make_async_copy(whbm[i].at[:, pl.ds(128*eh, 128)], raw_s.at[i, eh], sem.at[2*i + eh])

    def w1copy(j):
        f0, f1 = W1_SPLIT[j], W1_SPLIT[j + 1]
        return pltpu.make_async_copy(w1_hbm.at[:, pl.ds(f0, f1 - f0)], w1_s.at[:, pl.ds(f0, f1 - f0)], sem.at[32 + j])

    def xcopy(b0, nblk, k):
        return pltpu.make_async_copy(xT_hbm.at[:, pl.ds(b0*BLK, nblk*BLK)], xT_s.at[:, pl.ds(b0*BLK, nblk*BLK)], sem.at[10 + k])

    def xcopy_mid(i):
        off = (3 + 6*i) * BLK
        if not isinstance(i, int):
            off = pl.multiple_of(off, BLK)
        return pltpu.make_async_copy(xT_hbm.at[:, pl.ds(off, 6*BLK)], xT_s.at[:, pl.ds(off, 6*BLK)], sem.at[11 + i])

    def outcopy(c):
        off = c * BLK if isinstance(c, int) else pl.multiple_of(c * BLK, BLK)
        return pltpu.make_async_copy(outT_s.at[:, pl.ds(off, BLK)], outT_hbm.at[:, pl.ds(off, BLK)], sem.at[16 + c])

    ocopy = pltpu.make_async_copy(woT_hbm, woT_s, sem.at[6])
    w2copy = pltpu.make_async_copy(w2T_hbm, w2T_s, sem.at[8])

    xcopy(0, 3, 0).start()
    for j in range(3):
        w1copy(j).start()
    xcopy_mid(0).start(); xcopy_mid(1).start(); xcopy(15, 1, 3).start()
    for i in range(3):
        wcopy(i, 0).start(); wcopy(i, 1).start()
    ocopy.start(); w2copy.start()

    tok = {}

    def set_token(val):
        tok['z'] = pltpu.bitcast(val, u32) & pltpu.bitcast(R_s[0:8, 0:128], u32)

    def deint(i, dst, m):
        w32 = raw_s.bitcast(u32)
        for eh in range(2):
            a = w32[i, eh, pl.ds(m, D, stride=8), :]
            lo = pltpu.bitcast(pltpu.bitcast(a << 16, f32).astype(bf16), u32)
            hi = pltpu.bitcast(pltpu.bitcast(a & jnp.uint32(0xFFFF0000), f32).astype(bf16), u32)
            dst[2*m, :, 128*eh:128*(eh+1)] = lo
            dst[2*m+1, :, 128*eh:128*(eh+1)] = hi

    def rows_of(ref):
        return lambda h, a, b: _bf(ref[h, a//2:b//2, :])

    def pre_rem(dst, lhs, rhs, m, nd):
        Rt = jnp.concatenate([jax.lax.dot_general(rhs(h, DU, D), lhs(h, 0, nd), NT, preferred_element_type=f32)
                              for h in (2*m, 2*m+1)], axis=0)
        if nd % 128:
            Rt = jnp.concatenate([Rt, jnp.zeros((128, DP - D), f32)], axis=1)
        dst[:, 128*m:128*(m+1)] = pltpu.bitcast(Rt.T[0:nd].astype(bf16), u32)

    def pre_main(dst, lhs, rhs, h, nd):
        A = jax.lax.dot_general(lhs(h, 0, nd), rhs(h, 0, DU), NT, preferred_element_type=f32)
        dst[:, REM + DU*h:REM + DU*(h+1)] = pltpu.bitcast(A.astype(bf16), u32)

    def pre_A(m):
        pre_main(WK, rows_of(KD), rows_of(QD), 2*m + 1, DU)
        pre_rem(WQ, rows_of(QD), rows_of(KD), m, D)
        pre_main(WK, rows_of(KD), rows_of(QD), 2*m, DU)
        pre_rem(WK, rows_of(KD), rows_of(QD), m, DU)

    def pre_U(m):
        wo = lambda h, a, b: woT_s[h, a:b, :]
        pre_main(WV, rows_of(VD), wo, 2*m, DU)
        pre_main(WV, rows_of(VD), wo, 2*m + 1, DU)
        pre_rem(WV, rows_of(VD), wo, m, DU)
        for h in (2*m, 2*m + 1):
            Ut = jax.lax.dot_general(rows_of(VD)(h, DU, D), woT_s[h], NT, preferred_element_type=f32)
            WU[32*h:32*(h+1), 0:D] = pltpu.bitcast(Ut.astype(bf16), u32)

    def ln_block(c):
        t0 = c * BLK if isinstance(c, int) else pl.multiple_of(c * BLK, BLK)
        xb = xT_s[:, pl.ds(t0, BLK)].astype(f32)
        if 'z' in tok:
            xb = pltpu.bitcast(pltpu.bitcast(xb, u32) | jnp.concatenate([tok['z']] * (D // 8), axis=0), f32)
        mu = jnp.mean(xb, axis=0, keepdims=True)
        xc = xb - mu
        var = jnp.mean(xc * xc, axis=0, keepdims=True)
        xnT = xc * jax.lax.rsqrt(var + 1e-5)
        xn_s[pl.ds(t0, BLK), :] = jnp.concatenate([xnT, jnp.zeros((DP - D, BLK), f32)], axis=0).T

    def up_block(c, fa=0, fb=F):
        t0 = c * BLK if isinstance(c, int) else pl.multiple_of(c * BLK, BLK)
        h0 = c * (BLK // 2) if isinstance(c, int) else pl.multiple_of(c * (BLK // 2), BLK // 2)
        xb = xn_s[pl.ds(t0, BLK), 0:D].astype(bf16)
        h = jnp.dot(xb, _bf(W1[:, fa:fb]), preferred_element_type=f32)
        HID[pl.ds(h0, BLK // 2), fa:fb] = pltpu.bitcast(_silu(h).astype(bf16), u32)
        set_token(h[0:8, 0:128])

    def pack_w1(j):
        a, b = W1_SPLIT[j], W1_SPLIT[j + 1]
        W1[:, a:b] = pltpu.bitcast(w1_s[:, a:b], u32)

    R_s[...] = jnp.zeros((BLK, DP), f32)
    xcopy(0, 3, 0).wait()
    ln_block(0); ln_block(1)
    w1copy(0).wait(); pack_w1(0)
    up_block(0, W1_SPLIT[0], W1_SPLIT[1]); up_block(1, W1_SPLIT[0], W1_SPLIT[1])
    w1copy(1).wait(); pack_w1(1)
    up_block(0, W1_SPLIT[1], W1_SPLIT[2]); up_block(1, W1_SPLIT[1], W1_SPLIT[2])
    w1copy(2).wait(); pack_w1(2)
    up_block(0, W1_SPLIT[2], W1_SPLIT[3]); ln_block(2); up_block(1, W1_SPLIT[2], W1_SPLIT[3])

    def upbody(i, _):
        xcopy_mid(i).wait()
        for u in range(6):
            up_block(2 + 6*i + u)
            ln_block(2 + 6*i + u + 1)
        return None
    jax.lax.fori_loop(0, 2, upbody, None)

    xcopy(15, 1, 3).wait()
    for i in (0, 1):
        wcopy(i, 0).wait(); wcopy(i, 1).wait()
    tok.pop('z', None)
    up_block(14); ln_block(15); up_block(15)
    for m in range(8):
        deint(0, QD, m); deint(1, KD, m); pre_A(m)
    wcopy(2, 0).wait(); wcopy(2, 1).wait(); ocopy.wait(); w2copy.wait()
    for m in range(8):
        if m == 4:
            W2[...] = pltpu.bitcast(w2T_s[0:DU, :].T, u32)
        deint(2, VD, m); pre_U(m)

    def run_step(tag, h, hq, ngrp, row0, tok0, korder, qorder, tkeys, prev, hooks, dz=None, drow=None):
        hu = h[:, 0:DU]
        v = {}
        hid = _bf(HID[pl.ds(pl.multiple_of(tok0 // 2, 16), 16), :])
        YK = jnp.dot(hu, _bf(WK[...]), preferred_element_type=f32)
        v['YQ'] = jnp.dot(h[:, 0:D], _bf(WQ[...]), preferred_element_type=f32)
        qv = [v['YQ'][8*i:8*i+8] if i >= 0 else prev['q'] for i in qorder]
        Ql = jnp.concatenate([qv[u][:, 128*kp:128*(kp+1)] for kp in range(8) for u in range(5)], axis=0).astype(bf16)
        rowsB = []
        for t in range(5):
            rowsB += [tkeys[t], pltpu.roll(tkeys[t], 64, 1)]
        Bm = jnp.concatenate(rowsB + [jnp.zeros((48, 128), f32)], axis=0)
        S2 = jnp.dot(Ql, Bm.T.astype(bf16), preferred_element_type=f32)
        S2 = _block_transpose([S2[40*kp:40*(kp+1)] for kp in range(8)], 5)
        YV1 = jnp.dot(hu, _bf(WV[:, 0:V1[tag]]), preferred_element_type=f32)
        sk = _stack(YK, ngrp); v['sk'] = sk
        kk = jnp.concatenate([sk[i] if i >= 0 else prev['sk'] for i in korder], axis=0).astype(bf16)
        KT[...] = pltpu.bitcast(kk.T, u32)
        Sa = jnp.dot(hq, _bf(KT[:, 0:256]), preferred_element_type=f32)
        Sb = jnp.dot(hq[16:48], _bf(KT[:, 256:512]), preferred_element_type=f32)
        Sc = jnp.dot(hq[32:48], _bf(KT[:, 512:640]), preferred_element_type=f32)
        YV2 = jnp.dot(hu, _bf(WV[:, V1[tag]:V2[tag]]), preferred_element_type=f32)
        if tag == 'A':
            v['mb_prev'] = jnp.dot(prev['hid'][:, FS:], _bf(W2[FS//2:, :]), preferred_element_type=f32)
            ma = jnp.dot(hid[:, 0:FS], _bf(W2[0:FS//2, :]), preferred_element_type=f32)
        Pa, Pb, Pc, Pt = _softmax_pieces(Sa, Sb, Sc, S2)
        Pk = _block_transpose(Pt + [None, None, None], 8)
        Zt = jnp.dot(jnp.concatenate(Pk, axis=0).astype(bf16), Bm.astype(bf16), preferred_element_type=f32)
        if tag == 'B':
            Zl = jnp.concatenate([jnp.concatenate([Zt[40*kp:40*(kp+1)], dz[:, 128*kp:128*(kp+1)]], axis=0)
                                  for kp in range(8)], axis=1)
        else:
            Zl = jnp.concatenate([jnp.concatenate([Zt[40*kp:40*kp+24], Zt[40*kp+32:40*kp+40]], axis=0)
                                  for kp in range(8)], axis=1)
            v['dz'] = jnp.concatenate([Zt[40*kp+24:40*kp+32] for kp in range(8)], axis=1)
        YV = jnp.concatenate([YV1, YV2, jnp.dot(hu, _bf(WV[:, V2[tag]:]), preferred_element_type=f32)], axis=1)
        ot = jnp.dot(Zl.astype(bf16), _bf(WU[...]), preferred_element_type=f32)
        if tag == 'B':
            ot_tok, ot_mem = ot[0:32], ot[32:40]
            R_s[drow:drow+8, 0:D] = R_s[drow:drow+8, 0:D] + ot[40:48]
            if 'r' in hooks:
                hooks.pop('r')()
        else:
            ot_tok, ot_mem = jnp.concatenate([ot[0:24], jnp.zeros((8, D), f32)], axis=0), ot[24:32]
        sv = _stack(YV, ngrp); v['sv'] = sv
        vo = jnp.concatenate([sv[i] if i >= 0 else prev['sv'] for i in korder], axis=0).astype(bf16)
        oa = jnp.dot(Pa, vo[0:256], preferred_element_type=f32)
        ob = jnp.dot(Pb, vo[256:512], preferred_element_type=f32)
        oc = jnp.dot(Pc, vo[512:640], preferred_element_type=f32)
        hi = oa[16:48] + ob
        lastp = hi[16:32] + oc
        otok = jnp.concatenate([oa[0:8], hi[0:16], lastp[0:8]], axis=0)
        omem = lastp[8:16]
        if tag == 'B':
            ma = jnp.dot(hid[:, 0:FS], _bf(W2[0:FS//2, :]), preferred_element_type=f32)
        else:
            mb = jnp.dot(hid[:, FS:], _bf(W2[FS//2:, :]), preferred_element_type=f32)
        v['hid'] = hid
        att = otok[:, 0:D] + ot_tok
        R_s[row0:row0+32, DU:D] = att[:, DU:D]
        v['res'] = att[:, 0:DU] + ma
        if tag == 'A':
            R_s[row0:row0+32, 0:DU] = v['res'] + mb
        v['mem'] = jnp.concatenate([omem[:, 0:D] + ot_mem, jnp.zeros((8, DP - D), f32)], axis=1)
        return v

    def pair(r0, t0, mem, hooks, dz):
        g = [xn_s[pl.ds(t0 + r0 + 8*i, 8), :] for i in range(8)]
        tl = lambda a: a[:, DU:DP]
        hB = jnp.concatenate([g[0], g[4], g[1], g[2], g[3], mem], axis=0).astype(bf16)
        vB = run_step('B', hB, hB, 6, r0, t0 + r0, (5, 0, 2, 3, 4), (0, 2, 3, 4, 5),
                      [tl(mem), tl(g[0]), tl(g[1]), tl(g[2]), tl(g[3])], None, hooks, dz, (r0 - 8) % BLK)
        mem1 = vB['mem']
        hA = jnp.concatenate([g[5], g[6], g[7], mem1], axis=0).astype(bf16)
        hqA = jnp.concatenate([g[4], jnp.zeros((8, DP), f32), g[5], g[6], g[7], mem1], axis=0).astype(bf16)
        prev = {'sk': vB['sk'][1], 'sv': vB['sv'][1], 'q': vB['YQ'][8:16], 'hid': vB['hid']}
        vA = run_step('A', hA, hqA, 4, r0 + 32, t0 + r0 + 32, (3, -1, 0, 1, 2), (-1, 0, 1, 2, 3),
                      [tl(mem1), tl(g[4]), tl(g[5]), tl(g[6]), tl(g[7])], prev, hooks)
        R_s[r0:r0+32, 0:DU] = vB['res'] + vA['mb_prev']
        return vA['mem'], vA['dz']

    def down_tail(c):
        h0 = c * (BLK // 2) if isinstance(c, int) else pl.multiple_of(c * (BLK // 2), BLK // 2)
        return jax.lax.dot_general(w2T_s[DU:D, :], _bf(HID[pl.ds(h0, BLK // 2), :]), NT, preferred_element_type=f32)

    def out_block(c, rT, dt):
        off = c * BLK if isinstance(c, int) else pl.multiple_of(c * BLK, BLK)
        xb = xT_s[:, pl.ds(off, BLK)].astype(f32)
        outT_s[0:DU, pl.ds(off, BLK)] = (xb[0:DU] + rT[0:DU]).astype(bf16)
        outT_s[DU:D, pl.ds(off, BLK)] = (xb[DU:D] + rT[DU:D] + dt).astype(bf16)

    def body(c, carry):
        mem, dz = carry
        t0 = pl.multiple_of(c * BLK, BLK)
        cp = jnp.maximum(c - 1, 0)
        st = {}

        def transpose_prev():
            st['rT'] = R_s[...].T[0:D]

        mem, dz = pair(0, t0, mem, {'r': transpose_prev}, dz)
        out_block(cp, st['rT'], down_tail(cp))
        mem, dz = pair(64, t0, mem, {}, dz)

        @pl.when(c > 0)
        def _():
            outcopy(c - 1).start()
        return mem, dz

    mem0 = jnp.concatenate([mem_ref[...].astype(f32), jnp.zeros((MEM, DP - D), f32)], axis=1)
    _, dz_last = jax.lax.fori_loop(0, NB, body, (mem0, jnp.zeros((8, 1024), f32)))

    zl = jnp.concatenate([dz_last, jnp.zeros((8, 1024), f32)], axis=0).astype(bf16)
    tail = jnp.dot(zl, _bf(WU[...]), preferred_element_type=f32)[0:8]
    dt = down_tail(NB - 1)
    R_s[BLK-8:BLK, 0:D] = R_s[BLK-8:BLK, 0:D] + tail
    out_block(NB - 1, R_s[...].T[0:D], dt)
    outcopy(NB - 1).start()
    for c in range(NB):
        outcopy(c).wait()


def _run(A_x, A_mem0, A_Wq, A_Wk, A_Wv, A_Wo, B_w1, B_w2):
    any_spec = pl.BlockSpec(memory_space=pl.ANY)
    V = pltpu.VMEM
    outT = pl.pallas_call(
        _kernel,
        out_shape=jax.ShapeDtypeStruct((D, S), bf16),
        in_specs=[any_spec, pl.BlockSpec(memory_space=pltpu.VMEM)] + [any_spec] * 6,
        out_specs=any_spec,
        scratch_shapes=[
            V((D, S), bf16), V((S, DP), f32),
            V((3, 2, D*H, 128), bf16),
            V((H, D//2, DH), u32), V((H, D//2, DH), u32), V((H, D//2, DH), u32),
            V((H, D, DH), bf16), V((D, F), bf16), V((D, F), bf16),
            V((DU//2, 7168), u32), V((DU//2, 7168), u32), V((D//2, F), u32), V((F//2, DU), u32),
            V((BLK, DP), f32), V((D, S), bf16), V((S//2, F), u32),
            V((DP//2, 640), u32), V((D//2, 1024), u32), V((512, D), u32),
            pltpu.SemaphoreType.DMA((40,)),
        ],
        compiler_params=pltpu.CompilerParams(vmem_limit_bytes=100 * 1024 * 1024,
                                             flags={'XLA_TPU_EVENLY_DISTRIBUTE_CRITICAL_NODES': True}),
    )(jnp.swapaxes(A_x[0], 0, 1), A_mem0[0], A_Wq.reshape(D*H, DH), A_Wk.reshape(D*H, DH), A_Wv.reshape(D*H, DH),
      jnp.swapaxes(A_Wo, 1, 2), B_w1, jnp.swapaxes(B_w2, 0, 1))
    return jnp.swapaxes(outT, 0, 1)[None]


@jax.jit
def pallas_parallel_sum__memory_aug_recurrent_mem_tr__dense_activation_silu__prompt_kernel(
    A_x: jax.Array,
    A_mem0: jax.Array,
    A_Wq: jax.Array,
    A_Wk: jax.Array,
    A_Wv: jax.Array,
    A_Wo: jax.Array,
    A_seg_len: jax.Array,
    B_x: jax.Array,
    B_w1: jax.Array,
    B_w2: jax.Array,
):
    del A_seg_len, B_x
    return _run(A_x, A_mem0, A_Wq, A_Wk, A_Wv, A_Wo, B_w1, B_w2)
```

```python
import jax
import jax.numpy as jnp
from jax.experimental import pallas as pl
from jax.experimental.pallas import tpu as pltpu

D = 448; DP = 512; DU = 384; H = 16; DH = 256; F = 1792; MEM = 8; S = 2048
BLK = 128; NB = S // BLK
f32 = jnp.float32; bf16 = jnp.bfloat16; u32 = jnp.uint32
SCALE = DH ** -0.5
NEG = -1e9 / SCALE
NT = (((1,), (1,)), ((), ()))
REM = 1024
W1_SPLIT = (0, 384, 1024, F)
FS = 768
V1 = {'A': 2048, 'B': 1536}
V2 = {'A': 5632, 'B': 6144}


def _bf(x):
    return pltpu.bitcast(x, bf16)


def _stack(Y, ngroups):
    outs = []
    for g in range(ngroups):
        rows = Y[8*g:8*g+8, :]
        tiles = []
        for m in range(8):
            R = rows[:, 128*m:128*(m+1)]
            for h, rr in ((2*m, R), (2*m+1, pltpu.roll(R, 64, 1))):
                tiles.append(jnp.concatenate([rows[:, REM + DU*h:REM + DU*(h+1)], rr], axis=1))
        outs.append(jnp.concatenate(tiles, axis=0))
    return outs


def _group_allreduce(x, op):
    lane = jax.lax.broadcasted_iota(jnp.int32, x.shape, 1)
    parts = [x] + [jnp.where((lane & 7) >= r, pltpu.roll(x, r, 1), pltpu.roll(x, 128 - (8 - r), 1)) for r in range(1, 8)]
    while len(parts) > 1:
        parts = [op(parts[i], parts[i + 1]) for i in range(0, len(parts), 2)]
    return parts[0]


def _softmax_pieces(Sa, Sb, Sc, S2):
    sub = jax.lax.broadcasted_iota(jnp.int32, (8, 128), 0)
    lane = jax.lax.broadcasted_iota(jnp.int32, (8, 128), 1)
    tri = (lane & 7) <= sub
    row_a = {0: 0, 1: 16, 2: 24, 3: 32, 4: 40}

    def piece(u, t):
        if t < 2:
            return Sa[row_a[u]:row_a[u]+8, 128*t:128*(t+1)]
        if t < 4:
            return Sb[8*(u-1):8*u, 128*(t-2):128*(t-1)]
        return Sc[8*(u-3):8*(u-2), :]

    T = {}; ms = []
    for u in range(5):
        m = None
        for t in range(5):
            if not (u == 4 or t == 0 or t - 1 <= u):
                continue
            s = piece(u, t) + S2[t][8*u:8*u+8]
            if u < 4 and t - 1 == u:
                s = jnp.where(tri, s, NEG)
            T[u, t] = s
            m = s if m is None else jnp.maximum(m, s)
        ms.append(m)
    Mx = _group_allreduce(jnp.concatenate(ms, axis=0), jnp.maximum)
    E = {}; sums = []
    for u in range(5):
        sm = None
        for t in range(5):
            if (u, t) in T:
                e = jnp.exp((T[u, t] - Mx[8*u:8*u+8]) * SCALE)
                E[u, t] = e
                sm = e if sm is None else sm + e
        sums.append(sm)
    inv = 1.0 / _group_allreduce(jnp.concatenate(sums, axis=0), jnp.add)
    z = jnp.zeros((8, 128), f32)

    def p(u, t):
        return E[u, t] * inv[8*u:8*u+8] if (u, t) in E else z

    Pa = jnp.concatenate([jnp.concatenate([p(0, 0), p(0, 1)], axis=1), jnp.zeros((8, 256), f32)] +
                         [jnp.concatenate([p(u, 0), p(u, 1)], axis=1) for u in (1, 2, 3, 4)], axis=0)
    Pb = jnp.concatenate([jnp.concatenate([p(u, 2), p(u, 3)], axis=1) for u in (1, 2, 3, 4)], axis=0)
    Pc = jnp.concatenate([p(u, 4) for u in (3, 4)], axis=0)
    Pt = [jnp.concatenate([p(u, t) for u in range(5)], axis=0) for t in range(5)]
    return Pa.astype(bf16), Pb.astype(bf16), Pc.astype(bf16), Pt


def _block_transpose(blocks, nout):
    shape = next(x for x in blocks if x is not None).shape
    lane = jax.lax.broadcasted_iota(jnp.int32, shape, 1)
    zero = jnp.zeros(shape, f32)
    cur = list(blocks)
    for s in (1, 2, 4):
        hi = ((lane >> 4) & s) != 0
        nxt = []
        for k in range(8):
            if s == 4 and k >= nout:
                nxt.append(None)
                continue
            a_, b_ = (cur[k], cur[k + s]) if k & s == 0 else (cur[k - s], cur[k])
            if a_ is None and b_ is None:
                nxt.append(None)
            elif k & s == 0:
                nxt.append(jnp.where(hi, zero if b_ is None else pltpu.roll(b_, 16 * s, 1), zero if a_ is None else a_))
            else:
                nxt.append(jnp.where(hi, zero if b_ is None else b_, zero if a_ is None else pltpu.roll(a_, 128 - 16 * s, 1)))
        cur = nxt
    return [zero if x is None else x for x in cur[0:nout]]


def _silu(h):
    return h * pl.reciprocal(1.0 + jnp.exp(-h), approx=True)


def _kernel(xT_hbm, mem_ref, wq_hbm, wk_hbm, wv_hbm, woT_hbm, w1_hbm, w2T_hbm, outT_hbm,
            xT_s, xn_s, raw_s, QD, KD, VD, woT_s, w1_s, w2T_s, WK, WV, W1, W2, R_s, outT_s, HID, KT, WQ, WU,
            sem):
    whbm = (wq_hbm, wk_hbm, wv_hbm)

    def wcopy(i, eh):
        return pltpu.make_async_copy(whbm[i].at[:, pl.ds(128*eh, 128)], raw_s.at[i, eh], sem.at[2*i + eh])

    def w1copy(j):
        f0, f1 = W1_SPLIT[j], W1_SPLIT[j + 1]
        return pltpu.make_async_copy(w1_hbm.at[:, pl.ds(f0, f1 - f0)], w1_s.at[:, pl.ds(f0, f1 - f0)], sem.at[32 + j])

    def xcopy(b0, nblk, k):
        return pltpu.make_async_copy(xT_hbm.at[:, pl.ds(b0*BLK, nblk*BLK)], xT_s.at[:, pl.ds(b0*BLK, nblk*BLK)], sem.at[10 + k])

    def xcopy_mid(i):
        off = (3 + 6*i) * BLK
        if not isinstance(i, int):
            off = pl.multiple_of(off, BLK)
        return pltpu.make_async_copy(xT_hbm.at[:, pl.ds(off, 6*BLK)], xT_s.at[:, pl.ds(off, 6*BLK)], sem.at[11 + i])

    def outcopy(c):
        off = c * BLK if isinstance(c, int) else pl.multiple_of(c * BLK, BLK)
        return pltpu.make_async_copy(outT_s.at[:, pl.ds(off, BLK)], outT_hbm.at[:, pl.ds(off, BLK)], sem.at[16 + c])

    ocopy = pltpu.make_async_copy(woT_hbm, woT_s, sem.at[6])
    w2copy = pltpu.make_async_copy(w2T_hbm, w2T_s, sem.at[8])

    xcopy(0, 3, 0).start()
    for j in range(3):
        w1copy(j).start()
    xcopy_mid(0).start(); xcopy_mid(1).start(); xcopy(15, 1, 3).start()
    for i in range(3):
        wcopy(i, 0).start(); wcopy(i, 1).start()
    ocopy.start(); w2copy.start()

    tok = {}

    def set_token(val):
        tok['z'] = pltpu.bitcast(val, u32) & pltpu.bitcast(R_s[0:8, 0:128], u32)

    def deint(i, dst, m):
        w32 = raw_s.bitcast(u32)
        for eh in range(2):
            a = w32[i, eh, pl.ds(m, D, stride=8), :]
            lo = pltpu.bitcast(pltpu.bitcast(a << 16, f32).astype(bf16), u32)
            hi = pltpu.bitcast(pltpu.bitcast(a & jnp.uint32(0xFFFF0000), f32).astype(bf16), u32)
            dst[2*m, :, 128*eh:128*(eh+1)] = lo
            dst[2*m+1, :, 128*eh:128*(eh+1)] = hi

    def rows_of(ref):
        return lambda h, a, b: _bf(ref[h, a//2:b//2, :])

    def pre_rem(dst, lhs, rhs, m, nd):
        Rt = jnp.concatenate([jax.lax.dot_general(rhs(h, DU, D), lhs(h, 0, nd), NT, preferred_element_type=f32)
                              for h in (2*m, 2*m+1)], axis=0)
        if nd % 128:
            Rt = jnp.concatenate([Rt, jnp.zeros((128, DP - D), f32)], axis=1)
        dst[:, 128*m:128*(m+1)] = pltpu.bitcast(Rt.T[0:nd].astype(bf16), u32)

    def pre_main(dst, lhs, rhs, h, nd):
        A = jax.lax.dot_general(lhs(h, 0, nd), rhs(h, 0, DU), NT, preferred_element_type=f32)
        dst[:, REM + DU*h:REM + DU*(h+1)] = pltpu.bitcast(A.astype(bf16), u32)

    def pre_A(m):
        pre_main(WK, rows_of(KD), rows_of(QD), 2*m + 1, DU)
        pre_rem(WQ, rows_of(QD), rows_of(KD), m, D)
        pre_main(WK, rows_of(KD), rows_of(QD), 2*m, DU)
        pre_rem(WK, rows_of(KD), rows_of(QD), m, DU)

    def pre_U(m):
        wo = lambda h, a, b: woT_s[h, a:b, :]
        pre_main(WV, rows_of(VD), wo, 2*m, DU)
        pre_main(WV, rows_of(VD), wo, 2*m + 1, DU)
        pre_rem(WV, rows_of(VD), wo, m, DU)
        for h in (2*m, 2*m + 1):
            Ut = jax.lax.dot_general(rows_of(VD)(h, DU, D), woT_s[h], NT, preferred_element_type=f32)
            WU[32*h:32*(h+1), 0:D] = pltpu.bitcast(Ut.astype(bf16), u32)

    def ln_block(c):
        t0 = c * BLK if isinstance(c, int) else pl.multiple_of(c * BLK, BLK)
        xb = xT_s[:, pl.ds(t0, BLK)].astype(f32)
        if 'z' in tok:
            xb = pltpu.bitcast(pltpu.bitcast(xb, u32) | jnp.concatenate([tok['z']] * (D // 8), axis=0), f32)
        mu = jnp.mean(xb, axis=0, keepdims=True)
        xc = xb - mu
        var = jnp.mean(xc * xc, axis=0, keepdims=True)
        xnT = xc * jax.lax.rsqrt(var + 1e-5)
        xn_s[pl.ds(t0, BLK), :] = jnp.concatenate([xnT, jnp.zeros((DP - D, BLK), f32)], axis=0).T

    def up_block(c, fa=0, fb=F):
        t0 = c * BLK if isinstance(c, int) else pl.multiple_of(c * BLK, BLK)
        h0 = c * (BLK // 2) if isinstance(c, int) else pl.multiple_of(c * (BLK // 2), BLK // 2)
        xb = xn_s[pl.ds(t0, BLK), 0:D].astype(bf16)
        h = jnp.dot(xb, _bf(W1[:, fa:fb]), preferred_element_type=f32)
        HID[pl.ds(h0, BLK // 2), fa:fb] = pltpu.bitcast(_silu(h).astype(bf16), u32)
        set_token(h[0:8, 0:128])

    def pack_w1(j):
        a, b = W1_SPLIT[j], W1_SPLIT[j + 1]
        W1[:, a:b] = pltpu.bitcast(w1_s[:, a:b], u32)

    R_s[...] = jnp.zeros((BLK, DP), f32)
    xcopy(0, 3, 0).wait()
    ln_block(0); ln_block(1)
    w1copy(0).wait(); pack_w1(0)
    up_block(0, W1_SPLIT[0], W1_SPLIT[1]); up_block(1, W1_SPLIT[0], W1_SPLIT[1])
    w1copy(1).wait(); pack_w1(1)
    up_block(0, W1_SPLIT[1], W1_SPLIT[2]); up_block(1, W1_SPLIT[1], W1_SPLIT[2])
    w1copy(2).wait(); pack_w1(2)
    up_block(0, W1_SPLIT[2], W1_SPLIT[3]); ln_block(2); up_block(1, W1_SPLIT[2], W1_SPLIT[3])

    def upbody(i, _):
        xcopy_mid(i).wait()
        for u in range(6):
            up_block(2 + 6*i + u)
            ln_block(2 + 6*i + u + 1)
        return None
    jax.lax.fori_loop(0, 2, upbody, None)

    xcopy(15, 1, 3).wait()
    for i in (0, 1):
        wcopy(i, 0).wait(); wcopy(i, 1).wait()
    tok.pop('z', None)
    up_block(14); ln_block(15); up_block(15)
    for m in range(8):
        deint(0, QD, m); deint(1, KD, m); pre_A(m)
    wcopy(2, 0).wait(); wcopy(2, 1).wait(); ocopy.wait(); w2copy.wait()
    for m in range(8):
        if m == 4:
            W2[...] = pltpu.bitcast(w2T_s[0:DU, :].T, u32)
        deint(2, VD, m); pre_U(m)

    def run_step(tag, h, hq, ngrp, row0, tok0, korder, qorder, tkeys, prev):
        hu = h[:, 0:DU]
        v = {}
        hid = _bf(HID[pl.ds(pl.multiple_of(tok0 // 2, 16), 16), :])
        YK = jnp.dot(hu, _bf(WK[...]), preferred_element_type=f32)
        v['YQ'] = jnp.dot(h[:, 0:D], _bf(WQ[...]), preferred_element_type=f32)
        qv = [v['YQ'][8*i:8*i+8] if i >= 0 else prev['q'] for i in qorder]
        Ql = jnp.concatenate([qv[u][:, 128*kp:128*(kp+1)] for kp in range(8) for u in range(5)], axis=0).astype(bf16)
        rowsB = []
        for t in range(5):
            rowsB += [tkeys[t], pltpu.roll(tkeys[t], 64, 1)]
        Bm = jnp.concatenate(rowsB + [jnp.zeros((48, 128), f32)], axis=0)
        S2 = jnp.dot(Ql, Bm.T.astype(bf16), preferred_element_type=f32)
        S2 = _block_transpose([S2[40*kp:40*(kp+1)] for kp in range(8)], 5)
        YV1 = jnp.dot(hu, _bf(WV[:, 0:V1[tag]]), preferred_element_type=f32)
        sk = _stack(YK, ngrp); v['sk'] = sk
        kk = jnp.concatenate([sk[i] if i >= 0 else prev['sk'] for i in korder], axis=0).astype(bf16)
        KT[...] = pltpu.bitcast(kk.T, u32)
        Sa = jnp.dot(hq, _bf(KT[:, 0:256]), preferred_element_type=f32)
        Sb = jnp.dot(hq[16:48], _bf(KT[:, 256:512]), preferred_element_type=f32)
        Sc = jnp.dot(hq[32:48], _bf(KT[:, 512:640]), preferred_element_type=f32)
        YV2 = jnp.dot(hu, _bf(WV[:, V1[tag]:V2[tag]]), preferred_element_type=f32)
        if tag == 'A':
            v['mb_prev'] = jnp.dot(prev['hid'][:, FS:], _bf(W2[FS//2:, :]), preferred_element_type=f32)
            ma = jnp.dot(hid[:, 0:FS], _bf(W2[0:FS//2, :]), preferred_element_type=f32)
        Pa, Pb, Pc, Pt = _softmax_pieces(Sa, Sb, Sc, S2)
        Pk = _block_transpose(Pt + [None, None, None], 8)
        Zt = jnp.dot(jnp.concatenate(Pk, axis=0).astype(bf16), Bm.astype(bf16), preferred_element_type=f32)
        if tag == 'B':
            Zl = jnp.concatenate([jnp.concatenate([Zt[40*kp:40*kp+24], Zt[40*kp+32:40*kp+40]], axis=0)
                                  for kp in range(8)], axis=1)
            v['dz'] = jnp.concatenate([Zt[40*kp+24:40*kp+32] for kp in range(8)], axis=1)
        else:
            Zl = jnp.concatenate([jnp.concatenate([Zt[40*kp:40*(kp+1)], prev['dz'][:, 128*kp:128*(kp+1)]], axis=0)
                                  for kp in range(8)], axis=1)
        YV = jnp.concatenate([YV1, YV2, jnp.dot(hu, _bf(WV[:, V2[tag]:]), preferred_element_type=f32)], axis=1)
        ot = jnp.dot(Zl.astype(bf16), _bf(WU[...]), preferred_element_type=f32)
        if tag == 'B':
            ot_tok, ot_mem = jnp.concatenate([ot[0:24], jnp.zeros((8, D), f32)], axis=0), ot[24:32]
        else:
            ot_tok, ot_mem = ot[0:32], ot[32:40]
            v['ot_prev'] = ot[40:48]
        sv = _stack(YV, ngrp); v['sv'] = sv
        vo = jnp.concatenate([sv[i] if i >= 0 else prev['sv'] for i in korder], axis=0).astype(bf16)
        oa = jnp.dot(Pa, vo[0:256], preferred_element_type=f32)
        ob = jnp.dot(Pb, vo[256:512], preferred_element_type=f32)
        oc = jnp.dot(Pc, vo[512:640], preferred_element_type=f32)
        hi = oa[16:48] + ob
        lastp = hi[16:32] + oc
        otok = jnp.concatenate([oa[0:8], hi[0:16], lastp[0:8]], axis=0)
        omem = lastp[8:16]
        if tag == 'B':
            ma = jnp.dot(hid[:, 0:FS], _bf(W2[0:FS//2, :]), preferred_element_type=f32)
        else:
            mb = jnp.dot(hid[:, FS:], _bf(W2[FS//2:, :]), preferred_element_type=f32)
        v['hid'] = hid
        att = otok[:, 0:D] + ot_tok
        if tag == 'A':
            R_s[row0:row0+32, DU:D] = att[:, DU:D]
            R_s[row0:row0+32, 0:DU] = att[:, 0:DU] + ma + mb
        else:
            v['att'] = att; v['ma'] = ma
        v['mem'] = jnp.concatenate([omem[:, 0:D] + ot_mem, jnp.zeros((8, DP - D), f32)], axis=1)
        return v

    def pair(r0, t0, mem):
        g = [xn_s[pl.ds(t0 + r0 + 8*i, 8), :] for i in range(8)]
        tl = lambda a: a[:, DU:DP]
        hB = jnp.concatenate([g[0], g[4], g[1], g[2], g[3], mem], axis=0).astype(bf16)
        vB = run_step('B', hB, hB, 6, r0, t0 + r0, (5, 0, 2, 3, 4), (0, 2, 3, 4, 5),
                      [tl(mem), tl(g[0]), tl(g[1]), tl(g[2]), tl(g[3])], None)
        mem1 = vB['mem']
        hA = jnp.concatenate([g[5], g[6], g[7], mem1], axis=0).astype(bf16)
        hqA = jnp.concatenate([g[4], jnp.zeros((8, DP), f32), g[5], g[6], g[7], mem1], axis=0).astype(bf16)
        prev = {'sk': vB['sk'][1], 'sv': vB['sv'][1], 'q': vB['YQ'][8:16], 'hid': vB['hid'], 'dz': vB['dz']}
        vA = run_step('A', hA, hqA, 4, r0 + 32, t0 + r0 + 32, (3, -1, 0, 1, 2), (-1, 0, 1, 2, 3),
                      [tl(mem1), tl(g[4]), tl(g[5]), tl(g[6]), tl(g[7])], prev)
        attB = vB['att'] + jnp.concatenate([jnp.zeros((24, D), f32), vA['ot_prev']], axis=0)
        R_s[r0:r0+32, DU:D] = attB[:, DU:D]
        R_s[r0:r0+32, 0:DU] = attB[:, 0:DU] + vB['ma'] + vA['mb_prev']
        return vA['mem']

    def down_tail(c):
        h0 = c * (BLK // 2) if isinstance(c, int) else pl.multiple_of(c * (BLK // 2), BLK // 2)
        return jax.lax.dot_general(w2T_s[DU:D, :], _bf(HID[pl.ds(h0, BLK // 2), :]), NT, preferred_element_type=f32)

    def out_block(c, rT, dt):
        off = c * BLK if isinstance(c, int) else pl.multiple_of(c * BLK, BLK)
        xb = xT_s[:, pl.ds(off, BLK)].astype(f32)
        outT_s[0:DU, pl.ds(off, BLK)] = (xb[0:DU] + rT[0:DU]).astype(bf16)
        outT_s[DU:D, pl.ds(off, BLK)] = (xb[DU:D] + rT[DU:D] + dt).astype(bf16)

    def body(c, mem):
        t0 = pl.multiple_of(c * BLK, BLK)
        cp = jnp.maximum(c - 1, 0)
        rT = R_s[...].T[0:D]
        mem = pair(0, t0, mem)
        out_block(cp, rT, down_tail(cp))
        mem = pair(64, t0, mem)

        @pl.when(c > 0)
        def _():
            outcopy(c - 1).start()
        return mem

    mem0 = jnp.concatenate([mem_ref[...].astype(f32), jnp.zeros((MEM, DP - D), f32)], axis=1)
    jax.lax.fori_loop(0, NB, body, mem0)

    out_block(NB - 1, R_s[...].T[0:D], down_tail(NB - 1))
    outcopy(NB - 1).start()
    for c in range(NB):
        outcopy(c).wait()


def _run(A_x, A_mem0, A_Wq, A_Wk, A_Wv, A_Wo, B_w1, B_w2):
    any_spec = pl.BlockSpec(memory_space=pl.ANY)
    V = pltpu.VMEM
    outT = pl.pallas_call(
        _kernel,
        out_shape=jax.ShapeDtypeStruct((D, S), bf16),
        in_specs=[any_spec, pl.BlockSpec(memory_space=pltpu.VMEM)] + [any_spec] * 6,
        out_specs=any_spec,
        scratch_shapes=[
            V((D, S), bf16), V((S, DP), f32),
            V((3, 2, D*H, 128), bf16),
            V((H, D//2, DH), u32), V((H, D//2, DH), u32), V((H, D//2, DH), u32),
            V((H, D, DH), bf16), V((D, F), bf16), V((D, F), bf16),
            V((DU//2, 7168), u32), V((DU//2, 7168), u32), V((D//2, F), u32), V((F//2, DU), u32),
            V((BLK, DP), f32), V((D, S), bf16), V((S//2, F), u32),
            V((DP//2, 640), u32), V((D//2, 1024), u32), V((512, D), u32),
            pltpu.SemaphoreType.DMA((40,)),
        ],
        compiler_params=pltpu.CompilerParams(vmem_limit_bytes=100 * 1024 * 1024,
                                             flags={'XLA_TPU_EVENLY_DISTRIBUTE_CRITICAL_NODES': True}),
    )(jnp.swapaxes(A_x[0], 0, 1), A_mem0[0], A_Wq.reshape(D*H, DH), A_Wk.reshape(D*H, DH), A_Wv.reshape(D*H, DH),
      jnp.swapaxes(A_Wo, 1, 2), B_w1, jnp.swapaxes(B_w2, 0, 1))
    return jnp.swapaxes(outT, 0, 1)[None]


@jax.jit
def pallas_parallel_sum__memory_aug_recurrent_mem_tr__dense_activation_silu__prompt_kernel(
    A_x: jax.Array,
    A_mem0: jax.Array,
    A_Wq: jax.Array,
    A_Wk: jax.Array,
    A_Wv: jax.Array,
    A_Wo: jax.Array,
    A_seg_len: jax.Array,
    B_x: jax.Array,
    B_w1: jax.Array,
    B_w2: jax.Array,
):
    del A_seg_len, B_x
    return _run(A_x, A_mem0, A_Wq, A_Wk, A_Wv, A_Wo, B_w1, B_w2)
```

```python
import jax
import jax.numpy as jnp
from jax.experimental import pallas as pl
from jax.experimental.pallas import tpu as pltpu

D = 448; DP = 512; DU = 384; H = 16; DH = 256; F = 1792; MEM = 8; S = 2048
BLK = 128; NB = S // BLK
f32 = jnp.float32; bf16 = jnp.bfloat16; u32 = jnp.uint32
SCALE = DH ** -0.5
NEG = -1e9 / SCALE
NT = (((1,), (1,)), ((), ()))
REM = 1024
W1_SPLIT = (0, 384, 1024, F)
FS = 768
V1 = {'A': 2048, 'B': 1536}
V2 = {'A': 5632, 'B': 6144}


def _bf(x):
    return pltpu.bitcast(x, bf16)


def _stack(Y, ngroups):
    outs = []
    for g in range(ngroups):
        rows = Y[8*g:8*g+8, :]
        tiles = []
        for m in range(8):
            R = rows[:, 128*m:128*(m+1)]
            for h, rr in ((2*m, R), (2*m+1, pltpu.roll(R, 64, 1))):
                tiles.append(jnp.concatenate([rows[:, REM + DU*h:REM + DU*(h+1)], rr], axis=1))
        outs.append(jnp.concatenate(tiles, axis=0))
    return outs


def _group_allreduce(x, op):
    lane = jax.lax.broadcasted_iota(jnp.int32, x.shape, 1)
    parts = [x] + [jnp.where((lane & 7) >= r, pltpu.roll(x, r, 1), pltpu.roll(x, 128 - (8 - r), 1)) for r in range(1, 8)]
    while len(parts) > 1:
        parts = [op(parts[i], parts[i + 1]) for i in range(0, len(parts), 2)]
    return parts[0]


def _softmax_pieces(Sa, Sb, Sc, S2):
    sub = jax.lax.broadcasted_iota(jnp.int32, (8, 128), 0)
    lane = jax.lax.broadcasted_iota(jnp.int32, (8, 128), 1)
    tri = (lane & 7) <= sub
    row_a = {0: 0, 1: 16, 2: 24, 3: 32, 4: 40}

    def piece(u, t):
        if t < 2:
            return Sa[row_a[u]:row_a[u]+8, 128*t:128*(t+1)]
        if t < 4:
            return Sb[8*(u-1):8*u, 128*(t-2):128*(t-1)]
        return Sc[8*(u-3):8*(u-2), :]

    T = {}; ms = []
    for u in range(5):
        m = None
        for t in range(5):
            if not (u == 4 or t == 0 or t - 1 <= u):
                continue
            s = piece(u, t) + S2[t][8*u:8*u+8]
            if u < 4 and t - 1 == u:
                s = jnp.where(tri, s, NEG)
            T[u, t] = s
            m = s if m is None else jnp.maximum(m, s)
        ms.append(m)
    Mx = _group_allreduce(jnp.concatenate(ms, axis=0), jnp.maximum)
    E = {}; sums = []
    for u in range(5):
        sm = None
        for t in range(5):
            if (u, t) in T:
                e = jnp.exp((T[u, t] - Mx[8*u:8*u+8]) * SCALE)
                E[u, t] = e
                sm = e if sm is None else sm + e
        sums.append(sm)
    inv = 1.0 / _group_allreduce(jnp.concatenate(sums, axis=0), jnp.add)
    z = jnp.zeros((8, 128), f32)

    def p(u, t):
        return E[u, t] * inv[8*u:8*u+8] if (u, t) in E else z

    Pa = jnp.concatenate([jnp.concatenate([p(0, 0), p(0, 1)], axis=1), jnp.zeros((8, 256), f32)] +
                         [jnp.concatenate([p(u, 0), p(u, 1)], axis=1) for u in (1, 2, 3, 4)], axis=0)
    Pb = jnp.concatenate([jnp.concatenate([p(u, 2), p(u, 3)], axis=1) for u in (1, 2, 3, 4)], axis=0)
    Pc = jnp.concatenate([p(u, 4) for u in (3, 4)], axis=0)
    Pt = [jnp.concatenate([p(u, t) for u in range(5)], axis=0) for t in range(5)]
    return Pa.astype(bf16), Pb.astype(bf16), Pc.astype(bf16), Pt


def _block_transpose(blocks, nout):
    shape = next(x for x in blocks if x is not None).shape
    lane = jax.lax.broadcasted_iota(jnp.int32, shape, 1)
    zero = jnp.zeros(shape, f32)
    cur = list(blocks)
    for s in (1, 2, 4):
        hi = ((lane >> 4) & s) != 0
        nxt = []
        for k in range(8):
            if s == 4 and k >= nout:
                nxt.append(None)
                continue
            a_, b_ = (cur[k], cur[k + s]) if k & s == 0 else (cur[k - s], cur[k])
            if a_ is None and b_ is None:
                nxt.append(None)
            elif k & s == 0:
                nxt.append(jnp.where(hi, zero if b_ is None else pltpu.roll(b_, 16 * s, 1), zero if a_ is None else a_))
            else:
                nxt.append(jnp.where(hi, zero if b_ is None else b_, zero if a_ is None else pltpu.roll(a_, 128 - 16 * s, 1)))
        cur = nxt
    return [zero if x is None else x for x in cur[0:nout]]


def _silu(h):
    return h * pl.reciprocal(1.0 + jnp.exp(-h), approx=True)


def _kernel(xT_hbm, mem_hbm, wq_hbm, wk_hbm, wv_hbm, woT_hbm, w1_hbm, w2T_hbm, outT_hbm,
            xT_s, xn_s, raw_s, QD, KD, VD, woT_s, w1_s, w2T_s, WK, WV, W1, W2, R_s, outT_s, HID, KT, WQ, WU, mem_s,
            sem):
    whbm = (wq_hbm, wk_hbm, wv_hbm)

    def wcopy(i, eh):
        return pltpu.make_async_copy(whbm[i].at[:, pl.ds(128*eh, 128)], raw_s.at[i, eh], sem.at[2*i + eh])

    def w1copy(j):
        f0, f1 = W1_SPLIT[j], W1_SPLIT[j + 1]
        return pltpu.make_async_copy(w1_hbm.at[:, pl.ds(f0, f1 - f0)], w1_s.at[:, pl.ds(f0, f1 - f0)], sem.at[32 + j])

    def xcopy(b0, nblk, k):
        return pltpu.make_async_copy(xT_hbm.at[:, pl.ds(b0*BLK, nblk*BLK)], xT_s.at[:, pl.ds(b0*BLK, nblk*BLK)], sem.at[10 + k])

    def xcopy_mid(i):
        off = (3 + 6*i) * BLK
        if not isinstance(i, int):
            off = pl.multiple_of(off, BLK)
        return pltpu.make_async_copy(xT_hbm.at[:, pl.ds(off, 6*BLK)], xT_s.at[:, pl.ds(off, 6*BLK)], sem.at[11 + i])

    def outcopy(c):
        off = c * BLK if isinstance(c, int) else pl.multiple_of(c * BLK, BLK)
        return pltpu.make_async_copy(outT_s.at[:, pl.ds(off, BLK)], outT_hbm.at[:, pl.ds(off, BLK)], sem.at[16 + c])

    memcopy = pltpu.make_async_copy(mem_hbm, mem_s, sem.at[7])
    ocopy = pltpu.make_async_copy(woT_hbm, woT_s, sem.at[6])
    w2copy = pltpu.make_async_copy(w2T_hbm, w2T_s, sem.at[8])

    xcopy(0, 3, 0).start()
    for j in range(3):
        w1copy(j).start()
    xcopy_mid(0).start(); xcopy_mid(1).start(); xcopy(15, 1, 3).start()
    for i in range(3):
        wcopy(i, 0).start(); wcopy(i, 1).start()
    ocopy.start(); w2copy.start(); memcopy.start()

    tok = {}

    def set_token(val):
        tok['z'] = pltpu.bitcast(val, u32) & pltpu.bitcast(R_s[0:8, 0:128], u32)

    def deint(i, dst, m):
        w32 = raw_s.bitcast(u32)
        for eh in range(2):
            a = w32[i, eh, pl.ds(m, D, stride=8), :]
            lo = pltpu.bitcast(pltpu.bitcast(a << 16, f32).astype(bf16), u32)
            hi = pltpu.bitcast(pltpu.bitcast(a & jnp.uint32(0xFFFF0000), f32).astype(bf16), u32)
            dst[2*m, :, 128*eh:128*(eh+1)] = lo
            dst[2*m+1, :, 128*eh:128*(eh+1)] = hi

    def rows_of(ref):
        return lambda h, a, b: _bf(ref[h, a//2:b//2, :])

    def pre_rem(dst, lhs, rhs, m, nd):
        Rt = jnp.concatenate([jax.lax.dot_general(rhs(h, DU, D), lhs(h, 0, nd), NT, preferred_element_type=f32)
                              for h in (2*m, 2*m+1)], axis=0)
        if nd % 128:
            Rt = jnp.concatenate([Rt, jnp.zeros((128, DP - D), f32)], axis=1)
        dst[:, 128*m:128*(m+1)] = pltpu.bitcast(Rt.T[0:nd].astype(bf16), u32)

    def pre_main(dst, lhs, rhs, h, nd):
        A = jax.lax.dot_general(lhs(h, 0, nd), rhs(h, 0, DU), NT, preferred_element_type=f32)
        dst[:, REM + DU*h:REM + DU*(h+1)] = pltpu.bitcast(A.astype(bf16), u32)

    def pre_A(m):
        pre_main(WK, rows_of(KD), rows_of(QD), 2*m + 1, DU)
        pre_rem(WQ, rows_of(QD), rows_of(KD), m, D)
        pre_main(WK, rows_of(KD), rows_of(QD), 2*m, DU)
        pre_rem(WK, rows_of(KD), rows_of(QD), m, DU)

    def pre_U(m):
        wo = lambda h, a, b: woT_s[h, a:b, :]
        pre_main(WV, rows_of(VD), wo, 2*m, DU)
        pre_main(WV, rows_of(VD), wo, 2*m + 1, DU)
        pre_rem(WV, rows_of(VD), wo, m, DU)
        for h in (2*m, 2*m + 1):
            Ut = jax.lax.dot_general(rows_of(VD)(h, DU, D), woT_s[h], NT, preferred_element_type=f32)
            WU[32*h:32*(h+1), 0:D] = pltpu.bitcast(Ut.astype(bf16), u32)

    def ln_block(c):
        t0 = c * BLK if isinstance(c, int) else pl.multiple_of(c * BLK, BLK)
        xb = xT_s[:, pl.ds(t0, BLK)].astype(f32)
        if 'z' in tok:
            xb = pltpu.bitcast(pltpu.bitcast(xb, u32) | jnp.concatenate([tok['z']] * (D // 8), axis=0), f32)
        mu = jnp.mean(xb, axis=0, keepdims=True)
        xc = xb - mu
        var = jnp.mean(xc * xc, axis=0, keepdims=True)
        xnT = xc * jax.lax.rsqrt(var + 1e-5)
        xn_s[pl.ds(t0, BLK), :] = jnp.concatenate([xnT, jnp.zeros((DP - D, BLK), f32)], axis=0).T

    def up_block(c, fa=0, fb=F):
        t0 = c * BLK if isinstance(c, int) else pl.multiple_of(c * BLK, BLK)
        h0 = c * (BLK // 2) if isinstance(c, int) else pl.multiple_of(c * (BLK // 2), BLK // 2)
        xb = xn_s[pl.ds(t0, BLK), 0:D].astype(bf16)
        h = jnp.dot(xb, _bf(W1[:, fa:fb]), preferred_element_type=f32)
        HID[pl.ds(h0, BLK // 2), fa:fb] = pltpu.bitcast(_silu(h).astype(bf16), u32)
        set_token(h[0:8, 0:128])

    def pack_w1(j):
        a, b = W1_SPLIT[j], W1_SPLIT[j + 1]
        W1[:, a:b] = pltpu.bitcast(w1_s[:, a:b], u32)

    R_s[...] = jnp.zeros((BLK, DP), f32)
    xcopy(0, 3, 0).wait()
    ln_block(0); ln_block(1)
    w1copy(0).wait(); pack_w1(0)
    up_block(0, W1_SPLIT[0], W1_SPLIT[1]); up_block(1, W1_SPLIT[0], W1_SPLIT[1])
    w1copy(1).wait(); pack_w1(1)
    up_block(0, W1_SPLIT[1], W1_SPLIT[2]); up_block(1, W1_SPLIT[1], W1_SPLIT[2])
    w1copy(2).wait(); pack_w1(2)
    up_block(0, W1_SPLIT[2], W1_SPLIT[3]); ln_block(2); up_block(1, W1_SPLIT[2], W1_SPLIT[3])

    def upbody(i, _):
        xcopy_mid(i).wait()
        for u in range(6):
            up_block(2 + 6*i + u)
            ln_block(2 + 6*i + u + 1)
        return None
    jax.lax.fori_loop(0, 2, upbody, None)

    xcopy(15, 1, 3).wait()
    for i in (0, 1):
        wcopy(i, 0).wait(); wcopy(i, 1).wait()
    tok.pop('z', None)
    up_block(14); ln_block(15); up_block(15)
    for m in range(8):
        deint(0, QD, m); deint(1, KD, m); pre_A(m)
    wcopy(2, 0).wait(); wcopy(2, 1).wait(); ocopy.wait(); w2copy.wait()
    for m in range(8):
        if m == 4:
            W2[...] = pltpu.bitcast(w2T_s[0:DU, :].T, u32)
        deint(2, VD, m); pre_U(m)

    def run_step(tag, h, hq, ngrp, row0, tok0, korder, qorder, tkeys, prev):
        hu = h[:, 0:DU]
        v = {}
        hid = _bf(HID[pl.ds(pl.multiple_of(tok0 // 2, 16), 16), :])
        YK = jnp.dot(hu, _bf(WK[...]), preferred_element_type=f32)
        v['YQ'] = jnp.dot(h[:, 0:D], _bf(WQ[...]), preferred_element_type=f32)
        qv = [v['YQ'][8*i:8*i+8] if i >= 0 else prev['q'] for i in qorder]
        Ql = jnp.concatenate([qv[u][:, 128*kp:128*(kp+1)] for kp in range(8) for u in range(5)], axis=0).astype(bf16)
        rowsB = []
        for t in range(5):
            rowsB += [tkeys[t], pltpu.roll(tkeys[t], 64, 1)]
        Bm = jnp.concatenate(rowsB + [jnp.zeros((48, 128), f32)], axis=0)
        S2 = jnp.dot(Ql, Bm.T.astype(bf16), preferred_element_type=f32)
        S2 = _block_transpose([S2[40*kp:40*(kp+1)] for kp in range(8)], 5)
        YV1 = jnp.dot(hu, _bf(WV[:, 0:V1[tag]]), preferred_element_type=f32)
        sk = _stack(YK, ngrp); v['sk'] = sk
        kk = jnp.concatenate([sk[i] if i >= 0 else prev['sk'] for i in korder], axis=0).astype(bf16)
        KT[...] = pltpu.bitcast(kk.T, u32)
        Sa = jnp.dot(hq, _bf(KT[:, 0:256]), preferred_element_type=f32)
        Sb = jnp.dot(hq[16:48], _bf(KT[:, 256:512]), preferred_element_type=f32)
        Sc = jnp.dot(hq[32:48], _bf(KT[:, 512:640]), preferred_element_type=f32)
        YV2 = jnp.dot(hu, _bf(WV[:, V1[tag]:V2[tag]]), preferred_element_type=f32)
        if tag == 'A':
            v['mb_prev'] = jnp.dot(prev['hid'][:, FS:], _bf(W2[FS//2:, :]), preferred_element_type=f32)
            ma = jnp.dot(hid[:, 0:FS], _bf(W2[0:FS//2, :]), preferred_element_type=f32)
        Pa, Pb, Pc, Pt = _softmax_pieces(Sa, Sb, Sc, S2)
        Pk = _block_transpose(Pt + [None, None, None], 8)
        Zt = jnp.dot(jnp.concatenate(Pk, axis=0).astype(bf16), Bm.astype(bf16), preferred_element_type=f32)
        if tag == 'B':
            Zl = jnp.concatenate([jnp.concatenate([Zt[40*kp:40*kp+24], Zt[40*kp+32:40*kp+40]], axis=0)
                                  for kp in range(8)], axis=1)
            v['dz'] = jnp.concatenate([Zt[40*kp+24:40*kp+32] for kp in range(8)], axis=1)
        else:
            Zl = jnp.concatenate([jnp.concatenate([Zt[40*kp:40*(kp+1)], prev['dz'][:, 128*kp:128*(kp+1)]], axis=0)
                                  for kp in range(8)], axis=1)
        YV = jnp.concatenate([YV1, YV2, jnp.dot(hu, _bf(WV[:, V2[tag]:]), preferred_element_type=f32)], axis=1)
        ot = jnp.dot(Zl.astype(bf16), _bf(WU[...]), preferred_element_type=f32)
        if tag == 'B':
            ot_tok, ot_mem = jnp.concatenate([ot[0:24], jnp.zeros((8, D), f32)], axis=0), ot[24:32]
        else:
            ot_tok, ot_mem = ot[0:32], ot[32:40]
            v['ot_prev'] = ot[40:48]
        sv = _stack(YV, ngrp); v['sv'] = sv
        vo = jnp.concatenate([sv[i] if i >= 0 else prev['sv'] for i in korder], axis=0).astype(bf16)
        oa = jnp.dot(Pa, vo[0:256], preferred_element_type=f32)
        ob = jnp.dot(Pb, vo[256:512], preferred_element_type=f32)
        oc = jnp.dot(Pc, vo[512:640], preferred_element_type=f32)
        hi = oa[16:48] + ob
        lastp = hi[16:32] + oc
        otok = jnp.concatenate([oa[0:8], hi[0:16], lastp[0:8]], axis=0)
        omem = lastp[8:16]
        if tag == 'B':
            ma = jnp.dot(hid[:, 0:FS], _bf(W2[0:FS//2, :]), preferred_element_type=f32)
        else:
            mb = jnp.dot(hid[:, FS:], _bf(W2[FS//2:, :]), preferred_element_type=f32)
        v['hid'] = hid
        att = otok[:, 0:D] + ot_tok
        if tag == 'A':
            R_s[row0:row0+32, DU:D] = att[:, DU:D]
            R_s[row0:row0+32, 0:DU] = att[:, 0:DU] + ma + mb
        else:
            v['att'] = att; v['ma'] = ma
        v['mem'] = jnp.concatenate([omem[:, 0:D] + ot_mem, jnp.zeros((8, DP - D), f32)], axis=1)
        return v

    def pair(r0, t0, mem):
        g = [xn_s[pl.ds(t0 + r0 + 8*i, 8), :] for i in range(8)]
        tl = lambda a: a[:, DU:DP]
        hB = jnp.concatenate([g[0], g[4], g[1], g[2], g[3], mem], axis=0).astype(bf16)
        vB = run_step('B', hB, hB, 6, r0, t0 + r0, (5, 0, 2, 3, 4), (0, 2, 3, 4, 5),
                      [tl(mem), tl(g[0]), tl(g[1]), tl(g[2]), tl(g[3])], None)
        mem1 = vB['mem']
        hA = jnp.concatenate([g[5], g[6], g[7], mem1], axis=0).astype(bf16)
        hqA = jnp.concatenate([g[4], jnp.zeros((8, DP), f32), g[5], g[6], g[7], mem1], axis=0).astype(bf16)
        prev = {'sk': vB['sk'][1], 'sv': vB['sv'][1], 'q': vB['YQ'][8:16], 'hid': vB['hid'], 'dz': vB['dz']}
        vA = run_step('A', hA, hqA, 4, r0 + 32, t0 + r0 + 32, (3, -1, 0, 1, 2), (-1, 0, 1, 2, 3),
                      [tl(mem1), tl(g[4]), tl(g[5]), tl(g[6]), tl(g[7])], prev)
        attB = vB['att'] + jnp.concatenate([jnp.zeros((24, D), f32), vA['ot_prev']], axis=0)
        R_s[r0:r0+32, DU:D] = attB[:, DU:D]
        R_s[r0:r0+32, 0:DU] = attB[:, 0:DU] + vB['ma'] + vA['mb_prev']
        return vA['mem']

    def down_tail(c):
        h0 = c * (BLK // 2) if isinstance(c, int) else pl.multiple_of(c * (BLK // 2), BLK // 2)
        return jax.lax.dot_general(w2T_s[DU:D, :], _bf(HID[pl.ds(h0, BLK // 2), :]), NT, preferred_element_type=f32)

    def out_block(c, rT, dt):
        off = c * BLK if isinstance(c, int) else pl.multiple_of(c * BLK, BLK)
        xb = xT_s[:, pl.ds(off, BLK)].astype(f32)
        outT_s[0:DU, pl.ds(off, BLK)] = (xb[0:DU] + rT[0:DU]).astype(bf16)
        outT_s[DU:D, pl.ds(off, BLK)] = (xb[DU:D] + rT[DU:D] + dt).astype(bf16)

    def body(c, mem):
        t0 = pl.multiple_of(c * BLK, BLK)
        cp = jnp.maximum(c - 1, 0)
        rT = R_s[...].T[0:D]
        mem = pair(0, t0, mem)
        out_block(cp, rT, down_tail(cp))
        mem = pair(64, t0, mem)

        @pl.when(c > 0)
        def _():
            outcopy(c - 1).start()
        return mem

    memcopy.wait()
    mem0 = jnp.concatenate([mem_s[...].astype(f32), jnp.zeros((MEM, DP - D), f32)], axis=1)
    jax.lax.fori_loop(0, NB, body, mem0)

    out_block(NB - 1, R_s[...].T[0:D], down_tail(NB - 1))
    outcopy(NB - 1).start()
    for c in range(NB):
        outcopy(c).wait()


def _run(A_x, A_mem0, A_Wq, A_Wk, A_Wv, A_Wo, B_w1, B_w2):
    any_spec = pl.BlockSpec(memory_space=pl.ANY)
    V = pltpu.VMEM
    outT = pl.pallas_call(
        _kernel,
        out_shape=jax.ShapeDtypeStruct((D, S), bf16),
        in_specs=[any_spec] * 8,
        out_specs=any_spec,
        scratch_shapes=[
            V((D, S), bf16), V((S, DP), f32),
            V((3, 2, D*H, 128), bf16),
            V((H, D//2, DH), u32), V((H, D//2, DH), u32), V((H, D//2, DH), u32),
            V((H, D, DH), bf16), V((D, F), bf16), V((D, F), bf16),
            V((DU//2, 7168), u32), V((DU//2, 7168), u32), V((D//2, F), u32), V((F//2, DU), u32),
            V((BLK, DP), f32), V((D, S), bf16), V((S//2, F), u32),
            V((DP//2, 640), u32), V((D//2, 1024), u32), V((512, D), u32), V((MEM, D), bf16),
            pltpu.SemaphoreType.DMA((40,)),
        ],
        compiler_params=pltpu.CompilerParams(vmem_limit_bytes=100 * 1024 * 1024,
                                             flags={'XLA_TPU_EVENLY_DISTRIBUTE_CRITICAL_NODES': True}),
    )(jnp.swapaxes(A_x[0], 0, 1), A_mem0[0], A_Wq.reshape(D*H, DH), A_Wk.reshape(D*H, DH), A_Wv.reshape(D*H, DH),
      jnp.swapaxes(A_Wo, 1, 2), B_w1, jnp.swapaxes(B_w2, 0, 1))
    return jnp.swapaxes(outT, 0, 1)[None]


@jax.jit
def pallas_parallel_sum__memory_aug_recurrent_mem_tr__dense_activation_silu__prompt_kernel(
    A_x: jax.Array,
    A_mem0: jax.Array,
    A_Wq: jax.Array,
    A_Wk: jax.Array,
    A_Wv: jax.Array,
    A_Wo: jax.Array,
    A_seg_len: jax.Array,
    B_x: jax.Array,
    B_w1: jax.Array,
    B_w2: jax.Array,
):
    del A_seg_len, B_x
    return _run(A_x, A_mem0, A_Wq, A_Wk, A_Wv, A_Wo, B_w1, B_w2)
```
